```python
import jax
import jax.numpy as jnp

def _softmax(x, axis=-1):
    return jax.nn.softmax(x, axis=axis)

def _gelu(x):
    return jax.nn.gelu(x, approximate=True)

def _silu(x):
    return jax.nn.silu(x)

def _sigmoid(x):
    return jax.nn.sigmoid(x)

def _layernorm(x, axis=-1, eps=1e-05):
    m = jnp.mean(x, axis=axis, keepdims=True)
    v = jnp.var(x, axis=axis, keepdims=True)
    return (x - m) / jnp.sqrt(v + eps)

def _scatter_add(tgt, idx, src, axis=0):
    return tgt.at[idx].add(src)

def _segment_sum(src, seg, n):
    return jax.ops.segment_sum(src, seg, n)

class _Rng:

    def __init__(self, key):
        self._k = key

    def _next(self):
        self._k, sub = jax.random.split(self._k)
        return sub

    def normal(self, shape):
        return jax.random.normal(self._next(), shape, dtype=jnp.bfloat16)

    def randint(self, lo, hi, shape):
        return jax.random.randint(self._next(), shape, lo, hi, dtype=jnp.int32)

    def uniform(self, shape, lo=0.0, hi=1.0):
        return jax.random.uniform(self._next(), shape, jnp.bfloat16, lo, hi)

    def permutation(self, n):
        return jax.random.permutation(self._next(), n)
kernel_name = 'concat_heads__ssm_conv_s4__memory_aug_recurrent_mem_tr__prompt'

def setup_inputs():
    _rng = _Rng(jax.random.key(int.from_bytes(__import__("os").urandom(4), "little")))
    _w = lambda a: (lambda t: t.astype(jnp.bfloat16) if jnp.issubdtype(t.dtype, jnp.floating) else t)(jnp.asarray(a))

    def _A_setup():
        B, L, D, N = (1, 2048, 640, 128)
        A_re = -jnp.exp((lambda *s: _rng.normal(s) * 0.05)(D, N))
        A_im = jnp.pi * (lambda *s: _rng.normal(s) * 0.05)(D, N)
        B_re = (lambda *s: _rng.normal(s) * 0.05)(D, N)
        B_im = (lambda *s: _rng.normal(s) * 0.05)(D, N)
        C_re = (lambda *s: _rng.normal(s) * 0.05)(D, N)
        C_im = (lambda *s: _rng.normal(s) * 0.05)(D, N)
        log_dt = (lambda *s: _rng.normal(s) * 0.05)(D) * 0.5 - 4.0
        Dskip = (lambda *s: _rng.normal(s) * 0.05)(D)
        return {'u': _w((lambda *s: _rng.normal(s) * 0.05)(B, L, D)), 'A_re': _w(A_re), 'A_im': _w(A_im), 'B_re': _w(B_re), 'B_im': _w(B_im), 'C_re': _w(C_re), 'C_im': _w(C_im), 'log_dt': _w(log_dt), 'Dskip': _w(Dskip)}
    _A_in = _A_setup()

    def _B_setup():
        B, S, Dm = (1, 2048, 640)
        H, Dh = (32, 128)
        M, seg = (8, 32)
        seg = min(seg, S)
        S = S // seg * seg
        return {'x': _w((lambda *s: _rng.normal(s) * 0.05)(B, S, Dm)), 'mem0': _w((lambda *s: _rng.normal(s) * 0.05)(B, M, Dm)), 'Wq': _w((lambda *s: _rng.normal(s) * 0.05)(Dm, H, Dh) * Dm ** (-0.5)), 'Wk': _w((lambda *s: _rng.normal(s) * 0.05)(Dm, H, Dh) * Dm ** (-0.5)), 'Wv': _w((lambda *s: _rng.normal(s) * 0.05)(Dm, H, Dh) * Dm ** (-0.5)), 'Wo': _w((lambda *s: _rng.normal(s) * 0.05)(H, Dh, Dm) * (H * Dh) ** (-0.5)), 'seg_len': seg}
    _B_in = _B_setup()
    return {'A_u': _A_in['u'], 'A_A_re': _A_in['A_re'], 'A_A_im': _A_in['A_im'], 'A_B_re': _A_in['B_re'], 'A_B_im': _A_in['B_im'], 'A_C_re': _A_in['C_re'], 'A_C_im': _A_in['C_im'], 'A_log_dt': _A_in['log_dt'], 'A_Dskip': _A_in['Dskip'], 'B_x': _B_in['x'], 'B_mem0': _B_in['mem0'], 'B_Wq': _B_in['Wq'], 'B_Wk': _B_in['Wk'], 'B_Wv': _B_in['Wv'], 'B_Wo': _B_in['Wo'], 'B_seg_len': _B_in['seg_len']}

def reference(A_u, A_A_re, A_A_im, A_B_re, A_B_im, A_C_re, A_C_im, A_log_dt, A_Dskip, B_x, B_mem0, B_Wq, B_Wk, B_Wv, B_Wo, B_seg_len):

    def _A_ref(u, A_re, A_im, B_re, B_im, C_re, C_im, log_dt, Dskip):
        Bsz, L, D = u.shape
        dt = jnp.exp(log_dt)[:, None]
        A = A_re + 1j * A_im
        Bc = B_re + 1j * B_im
        Cc = C_re + 1j * C_im
        logdA = dt * A
        dB = dt * Bc
        l = (lambda x, dt: x.astype(dt))(jnp.arange(L), A_re.dtype)
        P = jnp.exp(logdA[:, :, None] * l[None, None, :])
        K = jnp.einsum('dn,dnl,dn->dl', Cc, P, dB).real
        L2 = 2 * L
        Kp = jnp.pad(K, ((0, 0), (0, L)))
        up = (lambda x, *d: x.transpose(*d))(u, 0, 2, 1)
        up = jnp.pad(up, ((0, 0), (0, 0), (0, L)))
        Kf = (lambda x, axes=(-2, -1): jnp.fft.rfft2(x.astype(jnp.float32), axes=axes))(Kp[:, None, :], axes=(-2, -1))
        Uf = (lambda x, axes=(-2, -1): jnp.fft.rfft2(x.astype(jnp.float32), axes=axes))(up[:, :, None, :], axes=(-2, -1))
        Yf = Uf * Kf[None, :, :, :]
        y = (lambda x, s, axes=(-2, -1): jnp.fft.irfft2(x, s=s, axes=axes).astype(jnp.bfloat16))(Yf, (1, L2), axes=(-2, -1))[:, :, 0, :L]
        y = (lambda x, *d: x.transpose(*d))(y, 0, 2, 1) + u * Dskip[None, None, :]
        return y

    def _B_ref(x, mem0, Wq, Wk, Wv, Wo, seg_len):
        B, S, Dm = x.shape
        H, Dh = (Wq.shape[1], Wq.shape[2])
        M = mem0.shape[1]
        scale = Dh ** (-0.5)
        n_seg = S // seg_len
        L = M + seg_len
        idx = jnp.arange(L)
        mask = (idx[:, None] < M) | (idx[:, None] >= idx[None, :])
        mem = mem0
        outs = []
        for s in range(n_seg):
            xs = x[:, s * seg_len:(s + 1) * seg_len, :].copy()
            h = jnp.concatenate([mem, xs], axis=1)
            q = jnp.einsum('btd,dhe->bhte', h, Wq)
            k = jnp.einsum('btd,dhe->bhte', h, Wk)
            v = jnp.einsum('btd,dhe->bhte', h, Wv)
            scores = jnp.einsum('bhqe,bhke->bhqk', q, k) * scale
            scores = jnp.where(mask[None, None], scores, -1000000000.0)
            p = _softmax(scores, axis=-1)
            o = jnp.einsum('bhqk,bhke->bhqe', p, v)
            o = jnp.einsum('bhte,hed->btd', o, Wo)
            mem = o[:, :M, :].copy()
            outs.append(o[:, M:, :])
        return jnp.concatenate(outs, axis=1)
    a = _A_ref(A_u, A_A_re, A_A_im, A_B_re, A_B_im, A_C_re, A_C_im, A_log_dt, A_Dskip)
    b = _B_ref(B_x, B_mem0, B_Wq, B_Wk, B_Wv, B_Wo, B_seg_len)
    return jnp.concatenate([a, b], axis=-1)
```

```python
import functools

import jax
import jax.numpy as jnp
import ml_dtypes
import numpy as np
import jax.experimental.pallas as pl
import jax.experimental.pallas.tpu as pltpu

_T = 128
_NB = 16
_AB = 8


def _conv_constants(L):
    T = _T
    nc = L // T
    lr = np.arange(L).astype(np.float32).astype(ml_dtypes.bfloat16).astype(np.int64)
    a_list, start = [], []
    for c in range(nc):
        sub = lr[c * T:(c + 1) * T] - c * T
        step = int(np.gcd.reduce(sub[sub > 0]))
        assert 8 % step == 0
        start.append(len(a_list) * _NB)
        a_list += [(c, j) for j in range(0, 8, step)]
    start_last = len(a_list) * _NB
    row_of = {}
    for ai, (c, j) in enumerate(a_list):
        for b in range(_NB):
            row_of[c * T + j + 8 * b] = ai * _NB + b
    row_of[L] = start_last
    n_rows = start_last + _NB
    f = np.concatenate([np.arange(0, T, 2), np.arange(1, T, 2)]) + 0.5
    ang = np.pi * f[:, None] * np.arange(T)[None, :] / T
    F = np.concatenate([np.cos(ang), -np.sin(ang)], axis=0)
    G = np.concatenate([np.cos(ang), -np.sin(ang)], axis=0).T / T
    fe, fe_idx, win = [], [], []
    for c in range(nc):
        cols = np.array([row_of[int(v)] for v in lr[c * T:(c + 1) * T]]) - start[c]
        w = 16
        while w < cols.max() + 1:
            w *= 2
        assert start[c] + w <= n_rows and w <= T
        E = np.zeros((T, T))
        E[np.arange(T), cols] = 1.0
        m = F @ E
        for i, o in enumerate(fe):
            if np.array_equal(o, m):
                break
        else:
            fe.append(m)
            i = len(fe) - 1
        fe_idx.append(i)
        win.append(w)
    to_bf16 = lambda a: np.asarray(a, np.float32).astype(ml_dtypes.bfloat16)
    return dict(a_list=a_list, start=start, start_last=start_last, n_rows=n_rows, win=win,
                fe_idx=fe_idx, F=to_bf16(np.stack([F] + fe)), G=to_bf16(G))


def _cmul(ar, ai, br, bi):
    return ar * br - ai * bi, ar * bi + ai * br


def _kernel(u_ref, are_ref, aim_ref, bre_ref, bim_ref, cre_ref, cim_ref, ldt_ref, dsk_ref,
            x_ref, mem_ref, wq_ref, wk_ref, wv_ref, wo_ref, f_ref, g_ref,
            o_ref,
            wqkv, wos, hbuf, stage, xr_t, xi_t, yr_t, yi_t, kd, kh, uh, zb, sem,
            *, cst, seg, grp):
    f32, bf16 = jnp.float32, jnp.bfloat16
    L, D = u_ref.shape
    N = are_ref.shape[1]
    S, Dm = x_ref.shape
    M = mem_ref.shape[0]
    H, Dh = wq_ref.shape[1], wq_ref.shape[2]
    T = _T
    nc = L // T
    NG = H // grp
    LH = M + seg
    nn = (((1,), (0,)), ((), ()))
    nt = (((1,), (1,)), ((), ()))

    for wi, wr in enumerate((wq_ref, wk_ref, wv_ref)):
        w32 = wr.bitcast(jnp.uint32)
        for hp in range(H // 2):
            pltpu.make_async_copy(w32.at[:, hp, :], stage.at[wi, hp], sem.at[wi]).start()
    wo_copy = pltpu.make_async_copy(wo_ref.bitcast(jnp.uint32), wos, sem.at[3])
    wo_copy.start()

    a_list, start, win, fe_idx = cst["a_list"], cst["start"], cst["win"], cst["fe_idx"]
    n_ablk = len(a_list) // _AB
    dt_all = jnp.exp(ldt_ref[...].astype(f32)).astype(bf16).astype(f32)
    dsk_all = dsk_ref[...].astype(f32)
    for j in range(D // 128):
        cs = slice(j * 128, (j + 1) * 128)
        dt = dt_all[:, cs]
        tr = lambda r: r[cs, :].astype(f32).T
        ar, ai = dt * tr(are_ref), dt * tr(aim_ref)
        wr_, wi_ = _cmul(tr(cre_ref), tr(cim_ref), dt * tr(bre_ref), dt * tr(bim_ref))

        def zpow(p):
            e = jnp.exp(ar * p)
            return e * jnp.cos(ai * p), e * jnp.sin(ai * p)

        z1, z8, zT = zpow(1.0), zpow(8.0), zpow(float(T))
        zj = {1: z1}
        for q in range(2, 8):
            zj[q] = _cmul(*zj[q // 2], *zj[q - q // 2])
        wc = (wr_, wi_)
        for ai_idx, (c, q) in enumerate(a_list):
            if q == 0:
                if c > 0:
                    wc = _cmul(*wc, *zT)
                v = wc
            else:
                v = _cmul(*wc, *zj[q])
            xr_t[ai_idx] = v[0]
            xi_t[ai_idx] = v[1]
        last = jnp.sum(wc[0] * zT[0] - wc[1] * zT[1], axis=0, keepdims=True)
        rows = jax.lax.broadcasted_iota(jnp.int32, (_NB, 128), 0)
        kd[cst["start_last"]:, :] = jnp.where(rows == 0, last, 0.0)
        yb = {0: (jnp.ones_like(ar), jnp.zeros_like(ar)), 1: z8}
        for b in range(_NB):
            if b > 1:
                yb[b] = _cmul(*yb[b // 2], *yb[b - b // 2])
            yr_t[pl.ds(b, N, stride=_NB), :] = yb[b][0]
            yi_t[pl.ds(b, N, stride=_NB), :] = yb[b][1]

        def kblock(blk, carry):
            def body(n, acc):
                r = pl.multiple_of(n * _NB, _NB)
                yr, yi = yr_t[pl.ds(r, _NB), :], yi_t[pl.ds(r, _NB), :]
                out = []
                for a in range(_AB):
                    xr = xr_t[blk * _AB + a, pl.ds(n, 1), :]
                    xi = xi_t[blk * _AB + a, pl.ds(n, 1), :]
                    out.append(acc[a] + (xr * yr - xi * yi))
                return tuple(out)
            acc = jax.lax.fori_loop(0, N, body, tuple(jnp.zeros((_NB, 128), f32) for _ in range(_AB)),
                                    unroll=4)
            for a in range(_AB):
                kd[pl.ds(pl.multiple_of((blk * _AB + a) * _NB, _NB), _NB), :] = acc[a]
            return carry
        jax.lax.fori_loop(0, n_ablk, kblock, 0)

        prev = None
        for c in range(nc):
            w = win[c]
            kh[c] = jax.lax.dot_general(f_ref[1 + fe_idx[c], :, :w], kd[start[c]:start[c] + w, :].astype(bf16),
                                        nn, preferred_element_type=f32)
            cur = jax.lax.dot_general(f_ref[0], u_ref[c * T:(c + 1) * T, cs], nn, preferred_element_type=f32)
            if prev is None:
                uh[c] = cur
            else:
                q = T // 2
                uh[c, 0:q] = cur[0:q] - prev[2 * q:3 * q]
                uh[c, q:2 * q] = cur[q:2 * q] + prev[3 * q:4 * q]
                uh[c, 2 * q:3 * q] = cur[2 * q:3 * q] + prev[0:q]
                uh[c, 3 * q:4 * q] = cur[3 * q:4 * q] - prev[q:2 * q]
            prev = cur

        def mac(fb, carry):
            r = pl.multiple_of(fb * 8, 8)
            cb = 4
            for c0 in range(0, nc, cb):
                acc = [None] * cb
                for d in range(c0 + cb):
                    kr, ki = kh[d, pl.ds(r, 8), :], kh[d, pl.ds(T + r, 8), :]
                    for c in range(max(c0, d), c0 + cb):
                        pr, pi = _cmul(kr, ki, uh[c - d, pl.ds(r, 8), :], uh[c - d, pl.ds(T + r, 8), :])
                        a_ = acc[c - c0]
                        acc[c - c0] = (pr, pi) if a_ is None else (a_[0] + pr, a_[1] + pi)
                for c in range(c0, c0 + cb):
                    zb[c, pl.ds(r, 8), :] = acc[c - c0][0]
                    zb[c, pl.ds(T + r, 8), :] = acc[c - c0][1]
            return carry
        jax.lax.fori_loop(0, T // 8, mac, 0)

        for c in range(nc):
            y = jax.lax.dot_general(g_ref[...], zb[c].astype(bf16), nn, preferred_element_type=f32)
            uu = u_ref[c * T:(c + 1) * T, cs].astype(f32)
            o_ref[c * T:(c + 1) * T, cs] = (y + uu * dsk_all[:, cs]).astype(bf16)

    for wi in range(3):
        pltpu.make_async_copy(stage.at[wi], stage.at[wi], sem.at[wi]).wait()

    def relayout(g, carry):
        for wi in range(3):
            for hp in range(grp // 2):
                xw = stage[wi, g * (grp // 2) + hp]
                lo = pltpu.bitcast(xw << 16, f32).astype(bf16)
                hi = pltpu.bitcast(xw & jnp.uint32(0xFFFF0000), f32).astype(bf16)
                c0 = ((2 * hp) * 3 + wi) * Dh
                c1 = ((2 * hp + 1) * 3 + wi) * Dh
                wqkv[g, :, c0:c0 + Dh] = pltpu.bitcast(lo, jnp.uint32)
                wqkv[g, :, c1:c1 + Dh] = pltpu.bitcast(hi, jnp.uint32)
        return carry
    jax.lax.fori_loop(0, NG, relayout, 0)
    wo_copy.wait()

    hbuf[0:M, :] = mem_ref[...].astype(f32)
    row = jax.lax.broadcasted_iota(jnp.int32, (LH, LH), 0)
    col = jax.lax.broadcasted_iota(jnp.int32, (LH, LH), 1)
    mask = (row < M) | (row >= col)
    scale = Dh ** -0.5

    def step(s, carry):
        r0 = pl.multiple_of(s * seg, seg)
        hbuf[M:LH, :] = x_ref[pl.ds(r0, seg), :].astype(f32)
        h = hbuf[...]

        def qkv(g):
            return jax.lax.dot_general(h, pltpu.bitcast(wqkv[g], bf16), nn, preferred_element_type=f32)

        def att(t):
            outs = []
            for hh in range(grp):
                q, k, v = (t[:, (3 * hh + i) * Dh:(3 * hh + i + 1) * Dh] for i in range(3))
                sc = jax.lax.dot_general(q, k, nt, preferred_element_type=f32) * scale
                sc = jnp.where(mask, sc, -1e9)
                e = jnp.exp(sc - jnp.max(sc, axis=-1, keepdims=True))
                p = e / jnp.sum(e, axis=-1, keepdims=True)
                outs.append(jax.lax.dot_general(p, v, nn, preferred_element_type=f32))
            return jnp.concatenate(outs, axis=1)

        def oproj(og, g):
            nr = grp * Dh // 2
            w = pltpu.bitcast(wos[g * nr:(g + 1) * nr, :], bf16)
            return jax.lax.dot_general(og, w, nn, preferred_element_type=f32)

        acc, ts, ogs = None, {}, {}
        for i in range(NG + 2):
            if i < NG:
                ts[i] = qkv(i)
            if 0 <= i - 1 < NG:
                ogs[i - 1] = att(ts.pop(i - 1))
            if 0 <= i - 2 < NG:
                t = oproj(ogs.pop(i - 2), i - 2)
                acc = t if acc is None else acc + t
        out = acc.astype(bf16)
        hbuf[0:M, :] = out[0:M].astype(f32)
        o_ref[pl.ds(r0, seg), D:] = out[M:LH]
        return carry
    jax.lax.fori_loop(0, S // seg, step, 0)


@functools.partial(jax.jit, static_argnames=("B_seg_len",))
def pallas_concat_heads__ssm_conv_s4__memory_aug_recurrent_mem_tr__prompt_kernel(
    A_u, A_A_re, A_A_im, A_B_re, A_B_im, A_C_re, A_C_im, A_log_dt, A_Dskip,
    B_x, B_mem0, B_Wq, B_Wk, B_Wv, B_Wo, B_seg_len,
):
    Bsz, L, D = A_u.shape
    N = A_A_re.shape[1]
    _, S, Dm = B_x.shape
    H, Dh = B_Wq.shape[1], B_Wq.shape[2]
    M = B_mem0.shape[1]
    assert Bsz == 1 and S == L and A_A_re.dtype == jnp.bfloat16
    grp = 4
    cst = _conv_constants(L)
    n_a = len(cst["a_list"])
    f32, u32 = jnp.float32, jnp.uint32
    vm = pl.BlockSpec(memory_space=pltpu.VMEM)
    hbm = pl.BlockSpec(memory_space=pl.ANY)
    out = pl.pallas_call(
        functools.partial(_kernel, cst=cst, seg=B_seg_len, grp=grp),
        out_shape=jax.ShapeDtypeStruct((L, D + Dm), jnp.bfloat16),
        in_specs=[vm] * 11 + [hbm] * 4 + [vm] * 2,
        out_specs=vm,
        scratch_shapes=[
            pltpu.VMEM((H // grp, Dm // 2, 3 * grp * Dh), u32),
            pltpu.VMEM((H * Dh // 2, Dm), u32),
            pltpu.VMEM((M + B_seg_len, Dm), f32),
            pltpu.VMEM((3, H // 2, Dm, Dh), u32),
            pltpu.VMEM((n_a, N, 128), f32),
            pltpu.VMEM((n_a, N, 128), f32),
            pltpu.VMEM((N * _NB, 128), f32),
            pltpu.VMEM((N * _NB, 128), f32),
            pltpu.VMEM((cst["n_rows"], 128), f32),
            pltpu.VMEM((L // _T, 2 * _T, 128), f32),
            pltpu.VMEM((L // _T, 2 * _T, 128), f32),
            pltpu.VMEM((L // _T, 2 * _T, 128), f32),
            pltpu.SemaphoreType.DMA((4,)),
        ],
        compiler_params=pltpu.CompilerParams(vmem_limit_bytes=120 * 1024 * 1024),
        name="s4_rmt",
    )(A_u.reshape(L, D), A_A_re, A_A_im, A_B_re, A_B_im, A_C_re, A_C_im,
      A_log_dt.reshape(1, D), A_Dskip.reshape(1, D),
      B_x.reshape(S, Dm), B_mem0.reshape(M, Dm), B_Wq, B_Wk, B_Wv, B_Wo.reshape(H * Dh, Dm),
      cst["F"], cst["G"])
    return out.reshape(1, L, D + Dm)
```

```python
import functools
import itertools

import jax
import jax.numpy as jnp
import ml_dtypes
import numpy as np
import jax.experimental.pallas as pl
import jax.experimental.pallas.tpu as pltpu

_T = 128
_NB = 32
_LAGS = (1, 3, 4)
_NA = 24
_SA, _SB = _NA + 1, _NB + 1


def _conv_constants(L):
    T = _T
    nc = L // T
    hb = _NB // 2
    lr = np.arange(L).astype(np.float32).astype(ml_dtypes.bfloat16).astype(np.int64)
    offs = []
    for m in range(nc // 2):
        sub = lr[2 * m * T:2 * (m + 1) * T] - 2 * m * T
        step = int(np.gcd.reduce(sub[sub > 0]))
        assert 8 % step == 0
        offs.append(list(range(0, 8, step)))
    start = [0]
    for c in range(nc):
        start.append(start[-1] + len(offs[c // 2]) * hb)
    start_last = start.pop()
    n_rows = start_last + hb
    a_list, row_of = [], {L: start_last}
    for m in range(nc // 2):
        for i, q in enumerate(offs[m]):
            dst = (start[2 * m] + i * hb, start[2 * m + 1] + i * hb)
            a_list.append((m, q, dst))
            for b in range(_NB):
                row_of[2 * m * T + q + 8 * b] = dst[b // hb] + b % hb
    a_list.append((nc // 2, 0, (start_last, None)))
    f = np.concatenate([np.arange(0, T, 2), np.arange(1, T, 2)]) + 0.5
    ang = np.pi * f[:, None] * np.arange(T)[None, :] / T
    F = np.concatenate([np.cos(ang), -np.sin(ang)], axis=0)
    G = np.concatenate([np.cos(ang), -np.sin(ang)], axis=0).T / T
    fe, fe_idx, win = [], [], []
    for c in range(nc):
        cols = np.array([row_of[int(v)] for v in lr[c * T:(c + 1) * T]]) - start[c]
        w = 16
        while w < cols.max() + 1:
            w *= 2
        assert start[c] + w <= n_rows and w <= T
        E = np.zeros((T, T))
        E[np.arange(T), cols] = 1.0
        m = F @ E
        for i, o in enumerate(fe):
            if np.array_equal(o, m):
                break
        else:
            fe.append(m)
            i = len(fe) - 1
        fe_idx.append(i)
        win.append(w)
    to_bf16 = lambda a: np.asarray(a, np.float32).astype(ml_dtypes.bfloat16)
    return dict(a_list=a_list, start=start, start_last=start_last, n_rows=n_rows, win=win,
                fe_idx=fe_idx, F=to_bf16(np.stack([F] + fe)), G=to_bf16(G))


def _cmul(ar, ai, br, bi):
    return ar * br - ai * bi, ar * bi + ai * br


def _kernel(are_ref, aim_ref, bre_ref, bim_ref, cre_ref, cim_ref, ldt_ref, dsk_ref, mem_ref, f_ref, g_ref,
            u_hbm, x_hbm, wq_hbm, wk_hbm, wv_hbm, wo_hbm,
            o_hbm,
            wqkv, wos, hbuf, stage, u_ref, x_ref, o_ref, par, xt, yt, kt, kd, kh, uh, zb, zero,
            sem, osem, *, cst, seg, grp):
    f32, bf16, u32 = jnp.float32, jnp.bfloat16, jnp.uint32
    L, D = u_ref.shape
    N = are_ref.shape[1]
    S, Dm = x_ref.shape
    M = mem_ref.shape[0]
    H, Dh = wq_hbm.shape[1], wq_hbm.shape[2]
    T = _T
    nc = L // T
    nt_ = D // 128
    NG = H // grp
    LH = M + seg
    n_seg = S // seg
    nn = (((1,), (0,)), ((), ()))
    nt = (((1,), (1,)), ((), ()))

    u_copy = pltpu.make_async_copy(u_hbm, u_ref, sem.at[4])
    u_copy.start()
    for wi, wr in enumerate((wq_hbm, wk_hbm, wv_hbm)):
        w32 = wr.bitcast(u32)
        for hp in range(H // 2):
            pltpu.make_async_copy(w32.at[:, hp, :], stage.at[wi, hp], sem.at[wi]).start()
    wo_copy = pltpu.make_async_copy(wo_hbm.bitcast(u32), wos, sem.at[3])
    wo_copy.start()
    x_copy = pltpu.make_async_copy(x_hbm, x_ref, sem.at[5])
    x_copy.start()

    a_list, start, win, fe_idx = cst["a_list"], cst["start"], cst["win"], cst["fe_idx"]
    dt_row = jnp.exp(ldt_ref[...].reshape(1, D).astype(f32)).astype(bf16).astype(f32)
    for j in range(nt_):
        cs = slice(j * 128, (j + 1) * 128)
        dt = jnp.broadcast_to(dt_row[:, cs], (N, 128)).T
        ld = lambda r: r[cs, :].astype(f32)
        par[0, cs] = dt * ld(are_ref)
        par[1, cs] = dt * ld(aim_ref)
        par[2, cs], par[3, cs] = _cmul(ld(cre_ref), ld(cim_ref), dt * ld(bre_ref), dt * ld(bim_ref))
    xt[...] = jnp.zeros(xt.shape, f32)

    def tables(g):
        r, slot = pl.multiple_of(g * 8, 8), g % 2
        ar, ai = par[0, pl.ds(r, 8), :], par[1, pl.ds(r, 8), :]

        def zpow(p):
            e = jnp.exp(ar * p)
            return e * jnp.cos(ai * p), e * jnp.sin(ai * p)

        zm = zpow(float(2 * T))
        zq = {1: zpow(1.0)}
        for q in range(2, 9):
            zq[q] = _cmul(*zq[q // 2], *zq[q - q // 2])
        wm = (par[2, pl.ds(r, 8), :], par[3, pl.ds(r, 8), :])
        for idx, (m, q, _) in enumerate(a_list):
            if q == 0 and m > 0:
                wm = _cmul(*wm, *zm)
            v = wm if q == 0 else _cmul(*wm, *zq[q])
            xt[slot, 0, pl.ds(idx, 8, stride=_SA), :] = v[0]
            xt[slot, 1, pl.ds(idx, 8, stride=_SA), :] = -v[1]
        yb = {0: (jnp.ones_like(ar), jnp.zeros_like(ar)), 1: zq[8]}
        for b in range(_NB):
            if b > 1:
                yb[b] = _cmul(*yb[b // 2], *yb[b - b // 2])
            yt[slot, 0, pl.ds(b, 8, stride=_SB), :] = yb[b][0]
            yt[slot, 1, pl.ds(b, 8, stride=_SB), :] = yb[b][1]

    def split(v):
        hi = pltpu.bitcast(pltpu.bitcast(v, u32) & u32(0xFFFF0000), f32)
        return hi, v - hi

    def mode_sum(g):
        slot = g % 2
        for i in range(8):
            lhs, rhs = [], []
            for part in range(2):
                xh, xl = split(xt[slot, part, i * _SA:i * _SA + _NA, :])
                yh, yl = split(yt[slot, part, i * _SB:i * _SB + _NB, :])
                lhs += [xh, xl, xh]
                rhs += [yh, yh, yl]
            kt[g, i * _SA:i * _SA + _NA, :] = jax.lax.dot_general(
                jnp.concatenate(lhs, axis=1), jnp.concatenate(rhs, axis=1), nt, preferred_element_type=f32)

    tables(0)

    def gen(g, carry):
        mode_sum(g - 1)
        tables(g)
        return carry
    jax.lax.fori_loop(1, D // 8, gen, 0)
    mode_sum(D // 8 - 1)

    u_copy.wait()

    def dft(j, carry):
        cs = pl.ds(pl.multiple_of(j * 128, 128), 128)
        hb = _NB // 2
        for idx, (_, _, dst) in enumerate(a_list):
            v = kt[pl.ds(j * 16, 16), pl.ds(idx, 8, stride=_SA), :].reshape(128, _NB).T
            if dst[1] is None:
                first = jax.lax.broadcasted_iota(jnp.int32, (hb, 128), 0) == 0
                kd[dst[0]:dst[0] + hb, :] = jnp.where(first, v[:hb], 0.0).astype(bf16)
            else:
                kd[dst[0]:dst[0] + hb, :] = v[:hb].astype(bf16)
                kd[dst[1]:dst[1] + hb, :] = v[hb:].astype(bf16)
        prev = None
        for c in range(nc):
            cur = jax.lax.dot_general(f_ref[0], u_ref[c * T:(c + 1) * T, cs], nn, preferred_element_type=f32)
            if prev is None:
                uh[j, c] = cur
            else:
                q = T // 2
                uh[j, c, 0:q] = cur[0:q] - prev[2 * q:3 * q]
                uh[j, c, q:2 * q] = cur[q:2 * q] + prev[3 * q:4 * q]
                uh[j, c, 2 * q:3 * q] = cur[2 * q:3 * q] + prev[0:q]
                uh[j, c, 3 * q:4 * q] = cur[3 * q:4 * q] - prev[q:2 * q]
            prev = cur
        for c in range(nc):
            w = win[c]
            kh[j, c] = jax.lax.dot_general(f_ref[1 + fe_idx[c], :, :w], kd[start[c]:start[c] + w, :],
                                           nn, preferred_element_type=f32)
        return carry
    jax.lax.fori_loop(0, nt_, dft, 0)

    n_fb = T // 8

    def after(v, tick):
        return v if tick is None else pltpu.bitcast(pltpu.bitcast(v, u32) | tick, f32)

    def mac(j, fb):
        r = pl.multiple_of(fb * 8, 8)
        cb = 4
        for c0 in range(0, nc, cb):
            acc = [None] * cb
            for d in range(c0 + cb):
                tick = yield
                kr, ki = after(kh[j, d, pl.ds(r, 8), :], tick), after(kh[j, d, pl.ds(T + r, 8), :], tick)
                for c in range(max(c0, d), c0 + cb):
                    pr, pi = _cmul(kr, ki, uh[j, c - d, pl.ds(r, 8), :], uh[j, c - d, pl.ds(T + r, 8), :])
                    a_ = acc[c - c0]
                    acc[c - c0] = (pr, pi) if a_ is None else (a_[0] + pr, a_[1] + pi)
            for c in range(c0, c0 + cb):
                zb[j, c, pl.ds(r, 8), :] = acc[c - c0][0]
                zb[j, c, pl.ds(T + r, 8), :] = acc[c - c0][1]

    def inverse(c, j):
        yield
        cs = slice(j * 128, (j + 1) * 128)
        r = pl.multiple_of(c * T, T)
        y = jax.lax.dot_general(g_ref[...], zb[j, c].astype(bf16), nn, preferred_element_type=f32)
        skip = u_ref[pl.ds(r, T), cs].astype(f32) * dsk_ref[...].reshape(1, D)[:, cs].astype(f32)
        o_ref[pl.ds(r, T), cs] = (y + skip).astype(bf16)

    for wi in range(3):
        pltpu.make_async_copy(stage.at[wi], stage.at[wi], sem.at[wi]).wait()

    def relayout(g, carry):
        half = Dm // 2
        for wi in range(3):
            for hp in range(grp // 2):
                ev = stage[wi, g * (grp // 2) + hp, pl.ds(0, half, stride=2), :]
                od = stage[wi, g * (grp // 2) + hp, pl.ds(1, half, stride=2), :]
                c0 = ((2 * hp) * 3 + wi) * Dh
                c1 = ((2 * hp + 1) * 3 + wi) * Dh
                wqkv[g, :, c0:c0 + Dh] = (ev & u32(0xFFFF)) | (od << 16)
                wqkv[g, :, c1:c1 + Dh] = (ev >> 16) | (od & u32(0xFFFF0000))
        return carry
    jax.lax.fori_loop(0, NG, relayout, 0)
    wo_copy.wait()
    x_copy.wait()

    hbuf[0:M, :] = mem_ref[...].astype(f32)
    zero[...] = jnp.zeros(zero.shape, u32)
    row = jax.lax.broadcasted_iota(jnp.int32, (LH, LH), 0)
    col = jax.lax.broadcasted_iota(jnp.int32, (LH, LH), 1)
    mask = (row < M) | (row >= col)
    scale = Dh ** -0.5

    def step(s, extra):
        r0 = pl.multiple_of(s * seg, seg)
        hbuf[M:LH, :] = x_ref[pl.ds(r0, seg), :].astype(f32)
        h = hbuf[...]

        def qkv(g):
            return jax.lax.dot_general(h, pltpu.bitcast(wqkv[g], bf16), nn, preferred_element_type=f32)

        def probs(t):
            res = []
            for hh in range(grp):
                q, k, v = (t[:, (3 * hh + i) * Dh:(3 * hh + i + 1) * Dh] for i in range(3))
                sc = jax.lax.dot_general(q, k, nt, preferred_element_type=f32) * scale
                sc = jnp.where(mask, sc, -1e9)
                e = jnp.exp(sc - jnp.max(sc, axis=-1, keepdims=True))
                res.append((e / jnp.sum(e, axis=-1, keepdims=True), v))
            return res

        def mix(res):
            return jnp.concatenate(
                [jax.lax.dot_general(p, v, nn, preferred_element_type=f32) for p, v in res], axis=1)

        def oproj(og, g):
            nr = grp * Dh // 2
            w = pltpu.bitcast(wos[g * nr:(g + 1) * nr, :], bf16)
            return jax.lax.dot_general(og, w, nn, preferred_element_type=f32)

        acc, ts, ps, ogs = None, {}, {}, {}
        la, lp, lo = _LAGS
        for i in range(NG + lo):
            if i < NG:
                ts[i] = qkv(i)
            if 0 <= i - la < NG:
                ps[i - la] = probs(ts.pop(i - la))
            if 0 <= i - lp < NG:
                ogs[i - lp] = mix(ps.pop(i - lp))
            extra(i, ts.get(i))
            if 0 <= i - lo < NG:
                t = oproj(ogs.pop(i - lo), i - lo)
                acc = t if acc is None else acc + t
        out = acc.astype(bf16)
        hbuf[0:M, :] = out[0:M].astype(f32)
        o_ref[pl.ds(r0, seg), D:] = out[M:LH]

    def interleave(gens, n_total, first, last):
        def chain():
            for g in gens:
                yield from g
        work = chain()
        next(work)

        def extra(i, t):
            if first <= i <= last:
                n, k = last - first + 1, i - first
                cnt = n_total * (k + 1) // n - n_total * k // n
                for m in range(cnt):
                    tick = None
                    if t is not None:
                        c0 = (m * (t.shape[1] // 128) // cnt) * 128
                        tick = pltpu.bitcast(t[0:8, c0:c0 + 128], u32) & zero[...]
                    try:
                        work.send(tick)
                    except StopIteration:
                        pass
        return extra

    s1 = n_seg - nc
    n_items = nt_ * n_fb
    per = -(-n_items // s1)

    def first(s, carry):
        items = [jnp.minimum(s * per + m, n_items - 1) for m in range(per)]
        step(s, interleave([mac(it // n_fb, it % n_fb) for it in items], per * 40, 0, NG - 1))
        return carry
    jax.lax.fori_loop(0, s1, first, 0)

    def out_copy(c):
        r = pl.multiple_of(c * T, T)
        return pltpu.make_async_copy(o_ref.at[pl.ds(r, T)], o_hbm.at[pl.ds(r, T)], osem.at[c])

    def finish(s, carry):
        c = s - s1
        step(s, interleave([inverse(c, j) for j in range(nt_)], nt_, NG + _LAGS[2] - nt_, NG + _LAGS[2] - 1))
        out_copy(c).start()
        return carry
    jax.lax.fori_loop(s1, n_seg, finish, 0)
    for c in range(nc):
        out_copy(c).wait()


@functools.partial(jax.jit, static_argnames=("B_seg_len",))
def pallas_concat_heads__ssm_conv_s4__memory_aug_recurrent_mem_tr__prompt_kernel(
    A_u, A_A_re, A_A_im, A_B_re, A_B_im, A_C_re, A_C_im, A_log_dt, A_Dskip,
    B_x, B_mem0, B_Wq, B_Wk, B_Wv, B_Wo, B_seg_len,
):
    Bsz, L, D = A_u.shape
    N = A_A_re.shape[1]
    _, S, Dm = B_x.shape
    H, Dh = B_Wq.shape[1], B_Wq.shape[2]
    M = B_mem0.shape[1]
    assert Bsz == 1 and S == L and A_A_re.dtype == jnp.bfloat16
    grp = 2
    cst = _conv_constants(L)
    assert len(cst["a_list"]) <= _NA and N == 128
    f32, u32 = jnp.float32, jnp.uint32
    vm = pl.BlockSpec(memory_space=pltpu.VMEM)
    hbm = pl.BlockSpec(memory_space=pl.ANY)
    out = pl.pallas_call(
        functools.partial(_kernel, cst=cst, seg=B_seg_len, grp=grp),
        out_shape=jax.ShapeDtypeStruct((L, D + Dm), jnp.bfloat16),
        in_specs=[vm] * 11 + [hbm] * 6,
        out_specs=hbm,
        scratch_shapes=[
            pltpu.VMEM((H // grp, Dm // 2, 3 * grp * Dh), u32),
            pltpu.VMEM((H * Dh // 2, Dm), u32),
            pltpu.VMEM((M + B_seg_len, Dm), f32),
            pltpu.VMEM((3, H // 2, Dm, Dh), u32),
            pltpu.VMEM((L, D), jnp.bfloat16),
            pltpu.VMEM((S, Dm), jnp.bfloat16),
            pltpu.VMEM((L, D + Dm), jnp.bfloat16),
            pltpu.VMEM((4, D, N), f32),
            pltpu.VMEM((2, 2, 8 * _SA, N), f32),
            pltpu.VMEM((2, 2, 8 * _SB, N), f32),
            pltpu.VMEM((D // 8, 8 * _SA, _NB), f32),
            pltpu.VMEM((cst["n_rows"], 128), jnp.bfloat16),
            pltpu.VMEM((D // 128, L // _T, 2 * _T, 128), f32),
            pltpu.VMEM((D // 128, L // _T, 2 * _T, 128), f32),
            pltpu.VMEM((D // 128, L // _T, 2 * _T, 128), f32),
            pltpu.VMEM((8, 128), u32),
            pltpu.SemaphoreType.DMA((6,)),
            pltpu.SemaphoreType.DMA((L // _T,)),
        ],
        compiler_params=pltpu.CompilerParams(vmem_limit_bytes=120 * 1024 * 1024),
        name="s4_rmt",
    )(A_A_re, A_A_im, A_B_re, A_B_im, A_C_re, A_C_im, A_log_dt, A_Dskip,
      B_mem0.reshape(M, Dm), cst["F"], cst["G"],
      A_u.reshape(L, D), B_x.reshape(S, Dm), B_Wq, B_Wk, B_Wv, B_Wo.reshape(H * Dh, Dm))
    return out.reshape(1, L, D + Dm)
```

```python
import functools
import math

import jax
import jax.numpy as jnp
import ml_dtypes
import numpy as np
import jax.experimental.pallas as pl
import jax.experimental.pallas.tpu as pltpu

_T = 128
_NB = 32
_LAGS = (1, 2, 3)
_NA = 24
_SA, _SB = _NA + 1, _NB + 1


def _conv_constants(L):
    T = _T
    nc = L // T
    hb = _NB // 2
    lr = np.arange(L).astype(np.float32).astype(ml_dtypes.bfloat16).astype(np.int64)
    offs = []
    for m in range(nc // 2):
        sub = lr[2 * m * T:2 * (m + 1) * T] - 2 * m * T
        step = int(np.gcd.reduce(sub[sub > 0]))
        assert 8 % step == 0
        offs.append(list(range(0, 8, step)))
    start = [0]
    for c in range(nc):
        start.append(start[-1] + len(offs[c // 2]) * hb)
    start_last = start.pop()
    n_rows = start_last + hb
    a_list, row_of = [], {L: start_last}
    for m in range(nc // 2):
        for i, q in enumerate(offs[m]):
            dst = (start[2 * m] + i * hb, start[2 * m + 1] + i * hb)
            a_list.append((m, q, dst))
            for b in range(_NB):
                row_of[2 * m * T + q + 8 * b] = dst[b // hb] + b % hb
    a_list.append((nc // 2, 0, (start_last, None)))
    f = np.concatenate([np.arange(0, T, 2), np.arange(1, T, 2)]) + 0.5
    ang = np.pi * f[:, None] * np.arange(T)[None, :] / T
    F = np.concatenate([np.cos(ang), -np.sin(ang)], axis=0)
    G = np.concatenate([np.cos(ang), -np.sin(ang)], axis=0).T / T
    mats, win = [F], []
    for c in range(nc):
        cols = np.array([row_of[int(v)] for v in lr[c * T:(c + 1) * T]]) - start[c]
        E = np.zeros((T, T))
        E[np.arange(T), cols] = 1.0
        m = F @ E
        if not np.array_equal(m, mats[-1]):
            mats.append(m)
        w = hb
        while w <= cols.max():
            w *= 2
        assert w <= T and start[c] + w <= n_rows
        win.append((len(mats) - 1, start[c], w))

    def pack(a):
        h = np.asarray(a, np.float32).astype(ml_dtypes.bfloat16).view(np.uint16).astype(np.uint32)
        return h[..., 0::2, :] | (h[..., 1::2, :] << 16)
    return dict(a_list=a_list, n_rows=n_rows, win=win,
                F=pack(np.stack(mats)), G=pack(G))


def _cmul(ar, ai, br, bi):
    return ar * br - ai * bi, ar * bi + ai * br


def _csqr(ar, ai):
    return (ar - ai) * (ar + ai), (ar + ar) * ai


def _kernel(are_ref, aim_ref, bre_ref, bim_ref, cre_ref, cim_ref, ldt_ref, dsk_ref, mem_ref, f_ref, g_ref,
            u_hbm, x_hbm, wq_hbm, wk_hbm, wv_hbm, wo_hbm,
            o_hbm,
            wqkv, wos, hbuf, stage, u_ref, x_ref, o_ref, par, zs0, zs1, xt0, xt1, yt0, yt1, kt, kd, kh, uh, zb, zero,
            sem, osem, *, cst, seg, grp):
    f32, bf16, u32 = jnp.float32, jnp.bfloat16, jnp.uint32
    L, D = u_ref.shape
    N = are_ref.shape[1]
    S, Dm = x_ref.shape
    M = mem_ref.shape[0]
    H, Dh = wq_hbm.shape[1], wq_hbm.shape[2]
    T = _T
    nc = L // T
    nt_ = D // 128
    NG = H // grp
    LH = M + seg
    n_seg = S // seg
    nn = (((1,), (0,)), ((), ()))
    nt = (((1,), (1,)), ((), ()))

    u_copy = pltpu.make_async_copy(u_hbm, u_ref, sem.at[4])
    u_copy.start()
    for wi, wr in enumerate((wq_hbm, wk_hbm, wv_hbm)):
        w32 = wr.bitcast(u32)
        for hp in range(H // 2):
            pltpu.make_async_copy(w32.at[:, hp, :], stage.at[wi, hp], sem.at[wi]).start()
    wo_copy = pltpu.make_async_copy(wo_hbm.bitcast(u32), wos, sem.at[3])
    wo_copy.start()
    x_copy = pltpu.make_async_copy(x_hbm, x_ref, sem.at[5])
    x_copy.start()

    a_list = cst["a_list"]
    dt_row = jnp.exp(ldt_ref[...].reshape(1, D).astype(f32)).astype(bf16).astype(f32)
    for j in range(nt_):
        cs = slice(j * 128, (j + 1) * 128)
        dt = jnp.broadcast_to(dt_row[:, cs], (N, 128)).T
        ld = lambda r: r[cs, :].astype(f32)
        par[0, cs] = dt * ld(are_ref)
        par[1, cs] = dt * ld(aim_ref)
        par[2, cs], par[3, cs] = _cmul(ld(cre_ref), ld(cim_ref), dt * ld(bre_ref), dt * ld(bim_ref))
    zs, xt, yt = (zs0, zs1), (xt0, xt1), (yt0, yt1)
    for r in xt:
        r[...] = jnp.zeros(r.shape, f32)
    n_grp = D // 8

    def bases(g, slot):
        r = pl.multiple_of(jnp.minimum(g, n_grp - 1) * 8, 8)
        ar, ai = par[0, pl.ds(r, 8), :], par[1, pl.ds(r, 8), :]
        e = jnp.exp(ar)
        zs[slot][0] = e * jnp.cos(ai)
        zs[slot][1] = e * jnp.sin(ai)

    def tables(g, slot):
        r = pl.multiple_of(jnp.minimum(g, n_grp - 1) * 8, 8)
        zq = {1: (zs[slot][0], zs[slot][1])}
        for q in range(2, 9):
            zq[q] = _cmul(*zq[q // 2], *zq[q - q // 2]) if q % 2 else _csqr(*zq[q // 2])
        yield zq[8][0]
        yb = {0: (jnp.ones((8, N), f32), jnp.zeros((8, N), f32)), 1: zq[8]}
        for b in range(_NB):
            if b > 1:
                yb[b] = _cmul(*yb[b // 2], *yb[b - b // 2]) if b % 2 else _csqr(*yb[b // 2])
            yt[slot][0, pl.ds(b, 8, stride=_SB), :] = yb[b][0]
            yt[slot][1, pl.ds(b, 8, stride=_SB), :] = yb[b][1]
            if b % 8 == 7:
                yield yb[b][1]
        zm = _csqr(*yb[_NB // 2])
        wm = (par[2, pl.ds(r, 8), :], par[3, pl.ds(r, 8), :])
        for idx, (m, q, _) in enumerate(a_list):
            if q == 0 and m > 0:
                wm = _cmul(*wm, *zm)
            v = wm if q == 0 else _cmul(*wm, *zq[q])
            xt[slot][0, pl.ds(idx, 8, stride=_SA), :] = v[0]
            xt[slot][1, pl.ds(idx, 8, stride=_SA), :] = -v[1]
            if idx % 7 == 6:
                yield v[1]

    def split(v):
        hi = pltpu.bitcast(pltpu.bitcast(v, u32) & u32(0xFFFF0000), f32)
        return hi, v - hi

    def after(v, tick):
        return v if tick is None else pltpu.bitcast(pltpu.bitcast(v, u32) | tick, f32)

    def tick_of(v):
        return pltpu.bitcast(v, u32) & zero[...]

    def mode_sum(g, slot, other=None):
        for i in range(8):
            tick = None if other is None else tick_of(next(other))
            lhs, rhs = [], []
            for part in range(2):
                xh, xl = split(xt[slot][part, i * _SA:i * _SA + _NA, :])
                y = [yt[slot][part, pl.ds(i * _SB + k, 8), :] for k in range(0, _NB, 8)]
                yh, yl = split(jnp.concatenate(y[:-1] + [after(y[-1], tick)], axis=0))
                lhs += [xh, xl, xh]
                rhs += [yh, yh, yl]
            kt[g, i * _SA:i * _SA + _NA, :] = jax.lax.dot_general(
                jnp.concatenate(lhs, axis=1), jnp.concatenate(rhs, axis=1), nt, preferred_element_type=f32)

    def regroup(j):
        hb = _NB // 2
        for idx, (_, _, dst) in enumerate(a_list):
            v = kt[pl.ds(j * 16, 16), pl.ds(idx, 8, stride=_SA), :].reshape(128, _NB).T
            if dst[1] is None:
                first = jax.lax.broadcasted_iota(jnp.int32, (hb, 128), 0) == 0
                kd[dst[0]:dst[0] + hb, :] = jnp.where(first, v[:hb], 0.0).astype(bf16)
            else:
                kd[dst[0]:dst[0] + hb, :] = v[:hb].astype(bf16)
                kd[dst[1]:dst[1] + hb, :] = v[hb:].astype(bf16)

    def forward(j):
        q, prev = T // 2, None
        cs = pl.ds(pl.multiple_of(j * 128, 128), 128)
        for c in range(nc):
            cur = jax.lax.dot_general(pltpu.bitcast(f_ref[0], bf16), u_ref[c * T:(c + 1) * T, cs],
                                      nn, preferred_element_type=f32)
            if prev is None:
                uh[j, c] = cur
            else:
                uh[j, c, 0:q] = cur[0:q] - prev[2 * q:3 * q]
                uh[j, c, q:2 * q] = cur[q:2 * q] + prev[3 * q:4 * q]
                uh[j, c, 2 * q:3 * q] = cur[2 * q:3 * q] + prev[0:q]
                uh[j, c, 3 * q:4 * q] = cur[3 * q:4 * q] - prev[q:2 * q]
            prev = cur
        for c, (mat, r0, w) in enumerate(cst["win"]):
            kh[j, c] = jax.lax.dot_general(pltpu.bitcast(f_ref[mat, :, :w], bf16), kd[r0:r0 + w, :],
                                           nn, preferred_element_type=f32)

    zero[...] = jnp.zeros(zero.shape, u32)
    bases(0, 0)
    bases(1, 1)
    list(tables(0, 0))

    def gen(i, carry):
        for k in range(2):
            g = 2 * i + k
            bases(g + 2, k)
            mode_sum(g, k, tables(g + 1, 1 - k))
        return carry
    jax.lax.fori_loop(0, n_grp // 2, gen, 0)
    u_copy.wait()

    def dft(j, carry):
        regroup(j)
        forward(j)
        return carry
    jax.lax.fori_loop(0, nt_, dft, 0)

    n_fb = T // 8

    def mac(j, fb):
        r = pl.multiple_of(fb * 8, 8)
        cb = 4
        for c0 in range(0, nc, cb):
            acc = [None] * cb
            for d in range(c0 + cb):
                tick = yield
                kr, ki = after(kh[j, d, pl.ds(r, 8), :], tick), after(kh[j, d, pl.ds(T + r, 8), :], tick)
                for c in range(max(c0, d), c0 + cb):
                    pr, pi = _cmul(kr, ki, uh[j, c - d, pl.ds(r, 8), :], uh[j, c - d, pl.ds(T + r, 8), :])
                    a_ = acc[c - c0]
                    acc[c - c0] = (pr, pi) if a_ is None else (a_[0] + pr, a_[1] + pi)
            for c in range(c0, c0 + cb):
                zb[j, c, pl.ds(r, 8), :] = acc[c - c0][0]
                zb[j, c, pl.ds(T + r, 8), :] = acc[c - c0][1]

    def inverse(c, j):
        yield
        cs = slice(j * 128, (j + 1) * 128)
        r = pl.multiple_of(c * T, T)
        y = jax.lax.dot_general(pltpu.bitcast(g_ref[...], bf16), zb[j, c].astype(bf16), nn, preferred_element_type=f32)
        skip = u_ref[pl.ds(r, T), cs].astype(f32) * dsk_ref[...].reshape(1, D)[:, cs].astype(f32)
        o_ref[pl.ds(r, T), cs] = (y + skip).astype(bf16)

    for wi in range(3):
        pltpu.make_async_copy(stage.at[wi], stage.at[wi], sem.at[wi]).wait()

    def relayout(g, carry):
        half = Dm // 2
        for wi in range(3):
            for hp in range(grp // 2):
                ev = stage[wi, g * (grp // 2) + hp, pl.ds(0, half, stride=2), :]
                od = stage[wi, g * (grp // 2) + hp, pl.ds(1, half, stride=2), :]
                c0 = ((2 * hp) * 3 + wi) * Dh
                c1 = ((2 * hp + 1) * 3 + wi) * Dh
                wqkv[g, :, c0:c0 + Dh] = (ev & u32(0xFFFF)) | (od << 16)
                wqkv[g, :, c1:c1 + Dh] = (ev >> 16) | (od & u32(0xFFFF0000))
        return carry
    jax.lax.fori_loop(0, NG, relayout, 0)
    wo_copy.wait()
    x_copy.wait()

    hbuf[0:M, :] = mem_ref[...].astype(f32)
    row = jax.lax.broadcasted_iota(jnp.int32, (LH, LH), 0)
    col = jax.lax.broadcasted_iota(jnp.int32, (LH, LH), 1)
    mask = (row < M) | (row >= col)
    scale = Dh ** -0.5

    def step(s, extra):
        r0 = pl.multiple_of(s * seg, seg)
        hbuf[M:LH, :] = x_ref[pl.ds(r0, seg), :].astype(f32)

        def qkv(g):
            outs = []
            for n0 in range(0, 3 * grp * Dh, 512):
                acc = None
                for k in range(Dm // 128):
                    w = pltpu.bitcast(wqkv[g, k * 64:(k + 1) * 64, n0:n0 + 512], bf16)
                    t = jax.lax.dot_general(hbuf[:, k * 128:(k + 1) * 128], w, nn, preferred_element_type=f32)
                    acc = t if acc is None else acc + t
                outs.append(acc)
            return jnp.concatenate(outs, axis=1)

        def probs(t):
            res = []
            for hh in range(grp):
                q, k, v = (t[:, (3 * hh + i) * Dh:(3 * hh + i + 1) * Dh] for i in range(3))
                sc = jax.lax.dot_general(q, k, nt, preferred_element_type=f32)
                sc = jnp.where(mask, sc, -1e9 / scale)
                e = jnp.exp2((sc - jnp.max(sc, axis=-1, keepdims=True)) * (scale * math.log2(math.e)))
                den = jnp.sum(e, axis=-1, keepdims=True)
                inv = pltpu.reciprocal(den, approx=True)
                res.append((e, v, inv * (2.0 - den * inv)))
            return res

        def mix(res):
            return jnp.concatenate(
                [jax.lax.dot_general(e, v, nn, preferred_element_type=f32) * inv for e, v, inv in res], axis=1)

        def oproj(og, g):
            nr = grp * Dh // 2
            w = pltpu.bitcast(wos[g * nr:(g + 1) * nr, :], bf16)
            return jax.lax.dot_general(og, w, nn, preferred_element_type=f32)

        acc, ts, ps, ogs = None, {}, {}, {}
        la, lp, lo = _LAGS
        for i in range(NG + lo):
            if i < NG:
                ts[i] = qkv(i)
            if 0 <= i - la < NG:
                ps[i - la] = probs(ts.pop(i - la))
            if 0 <= i - lp < NG:
                ogs[i - lp] = mix(ps.pop(i - lp))
            extra(i, ts.get(i))
            if 0 <= i - lo < NG:
                t = oproj(ogs.pop(i - lo), i - lo)
                acc = t if acc is None else acc + t
        extra(NG + lo, None)
        out = acc.astype(bf16)
        hbuf[0:M, :] = out[0:M].astype(f32)
        o_ref[pl.ds(r0, seg), D:] = out[M:LH]

    def interleave(gens, n_total, first, last):
        def chain():
            for g in gens:
                yield from g
        work = chain()
        next(work)

        def extra(i, t):
            if first <= i <= last:
                n, k = last - first + 1, i - first
                cnt = n_total * (k + 1) // n - n_total * k // n
                for m in range(cnt):
                    tick = None
                    if t is not None:
                        c0 = (m * (t.shape[1] // 128) // cnt) * 128
                        tick = tick_of(t[0:8, c0:c0 + 128])
                    try:
                        work.send(tick)
                    except StopIteration:
                        pass
        return extra

    s1 = n_seg - nc
    n_items = nt_ * n_fb
    per = -(-n_items // s1)

    def first(s, carry):
        items = [jnp.minimum(s * per + m, n_items - 1) for m in range(per)]
        step(s, interleave([mac(it // n_fb, it % n_fb) for it in items], per * 40, 0, NG - 1))
        return carry
    jax.lax.fori_loop(0, s1, first, 0)

    def out_copy(c):
        r = pl.multiple_of(c * T, T)
        return pltpu.make_async_copy(o_ref.at[pl.ds(r, T)], o_hbm.at[pl.ds(r, T)], osem.at[c])

    def finish(s, carry):
        c = s - s1
        step(s, interleave([inverse(c, j) for j in range(nt_)], nt_, NG + _LAGS[2] + 1 - nt_, NG + _LAGS[2]))
        out_copy(c).start()
        return carry
    jax.lax.fori_loop(s1, n_seg, finish, 0)
    for c in range(nc):
        out_copy(c).wait()


@functools.partial(jax.jit, static_argnames=("B_seg_len",))
def pallas_concat_heads__ssm_conv_s4__memory_aug_recurrent_mem_tr__prompt_kernel(
    A_u, A_A_re, A_A_im, A_B_re, A_B_im, A_C_re, A_C_im, A_log_dt, A_Dskip,
    B_x, B_mem0, B_Wq, B_Wk, B_Wv, B_Wo, B_seg_len,
):
    Bsz, L, D = A_u.shape
    N = A_A_re.shape[1]
    _, S, Dm = B_x.shape
    H, Dh = B_Wq.shape[1], B_Wq.shape[2]
    M = B_mem0.shape[1]
    assert Bsz == 1 and S == L and A_A_re.dtype == jnp.bfloat16
    grp = 4
    cst = _conv_constants(L)
    assert len(cst["a_list"]) <= _NA and N == 128
    f32, u32 = jnp.float32, jnp.uint32
    vm = pl.BlockSpec(memory_space=pltpu.VMEM)
    hbm = pl.BlockSpec(memory_space=pl.ANY)
    out = pl.pallas_call(
        functools.partial(_kernel, cst=cst, seg=B_seg_len, grp=grp),
        out_shape=jax.ShapeDtypeStruct((L, D + Dm), jnp.bfloat16),
        in_specs=[vm] * 11 + [hbm] * 6,
        out_specs=hbm,
        scratch_shapes=[
            pltpu.VMEM((H // grp, Dm // 2, 3 * grp * Dh), u32),
            pltpu.VMEM((H * Dh // 2, Dm), u32),
            pltpu.VMEM((M + B_seg_len, Dm), f32),
            pltpu.VMEM((3, H // 2, Dm, Dh), u32),
            pltpu.VMEM((L, D), jnp.bfloat16),
            pltpu.VMEM((S, Dm), jnp.bfloat16),
            pltpu.VMEM((L, D + Dm), jnp.bfloat16),
            pltpu.VMEM((4, D, N), f32),
            *[pltpu.VMEM((2, 8, N), f32)] * 2,
            *[pltpu.VMEM((2, 8 * _SA, N), f32)] * 2,
            *[pltpu.VMEM((2, 8 * _SB, N), f32)] * 2,
            pltpu.VMEM((D // 8, 8 * _SA, _NB), f32),
            pltpu.VMEM((cst["n_rows"], 128), jnp.bfloat16),
            pltpu.VMEM((D // 128, L // _T, 2 * _T, 128), f32),
            pltpu.VMEM((D // 128, L // _T, 2 * _T, 128), f32),
            pltpu.VMEM((D // 128, L // _T, 2 * _T, 128), f32),
            pltpu.VMEM((8, 128), u32),
            pltpu.SemaphoreType.DMA((6,)),
            pltpu.SemaphoreType.DMA((L // _T,)),
        ],
        compiler_params=pltpu.CompilerParams(vmem_limit_bytes=120 * 1024 * 1024),
        name="s4_rmt",
    )(A_A_re, A_A_im, A_B_re, A_B_im, A_C_re, A_C_im, A_log_dt, A_Dskip,
      B_mem0.reshape(M, Dm), cst["F"], cst["G"],
      A_u.reshape(L, D), B_x.reshape(S, Dm), B_Wq, B_Wk, B_Wv, B_Wo.reshape(H * Dh, Dm))
    return out.reshape(1, L, D + Dm)
```

```python
import functools
import math

import jax
import jax.numpy as jnp
import ml_dtypes
import numpy as np
import jax.experimental.pallas as pl
import jax.experimental.pallas.tpu as pltpu

_T = 128
_NB = 32
_LAGS = (1, 2, 3)
_X_HEAD = 2
_NA = 24
_SA, _SB = _NA + 1, _NB + 1


def _conv_constants(L):
    T = _T
    nc = L // T
    hb = _NB // 2
    lr = np.arange(L).astype(np.float32).astype(ml_dtypes.bfloat16).astype(np.int64)
    offs = []
    for m in range(nc // 2):
        sub = lr[2 * m * T:2 * (m + 1) * T] - 2 * m * T
        step = int(np.gcd.reduce(sub[sub > 0]))
        assert 8 % step == 0
        offs.append(list(range(0, 8, step)))
    start = [0]
    for c in range(nc):
        start.append(start[-1] + len(offs[c // 2]) * hb)
    start_last = start.pop()
    n_rows = start_last + hb
    a_list, row_of = [], {L: start_last}
    for m in range(nc // 2):
        for i, q in enumerate(offs[m]):
            dst = (start[2 * m] + i * hb, start[2 * m + 1] + i * hb)
            a_list.append((m, q, dst))
            for b in range(_NB):
                row_of[2 * m * T + q + 8 * b] = dst[b // hb] + b % hb
    a_list.append((nc // 2, 0, (start_last, None)))
    f = np.concatenate([np.arange(0, T, 2), np.arange(1, T, 2)]) + 0.5
    ang = np.pi * f[:, None] * np.arange(T)[None, :] / T
    F = np.concatenate([np.cos(ang), -np.sin(ang)], axis=0)
    G = np.concatenate([np.cos(ang), -np.sin(ang)], axis=0).T / T
    mats, win = [F], []
    for c in range(nc):
        cols = np.array([row_of[int(v)] for v in lr[c * T:(c + 1) * T]]) - start[c]
        E = np.zeros((T, T))
        E[np.arange(T), cols] = 1.0
        m = F @ E
        if not np.array_equal(m, mats[-1]):
            mats.append(m)
        w = hb
        while w <= cols.max():
            w *= 2
        assert w <= T and start[c] + w <= n_rows
        win.append((len(mats) - 1, start[c], w))

    def pack(a):
        h = np.asarray(a, np.float32).astype(ml_dtypes.bfloat16).view(np.uint16).astype(np.uint32)
        return h[..., 0::2, :] | (h[..., 1::2, :] << 16)
    return dict(a_list=a_list, n_rows=n_rows, win=win,
                F=pack(np.stack(mats)), G=pack(G))


def _cmul(ar, ai, br, bi):
    return ar * br - ai * bi, ar * bi + ai * br


def _csqr(ar, ai):
    return (ar - ai) * (ar + ai), (ar + ar) * ai


def _kernel(are_ref, aim_ref, bre_ref, bim_ref, cre_ref, cim_ref, ldt_ref, dsk_ref, mem_ref, f_ref, g_ref,
            u_hbm, x_hbm, wq_hbm, wk_hbm, wv_hbm, wo_hbm,
            o_hbm,
            wqkv, wos, hbuf, stage, u_ref, x_ref, o_ref, par, zs0, zs1, xt0, xt1, yt0, yt1, kt, kd, kh, uh, zb, zero,
            sem, osem, *, cst, seg, grp):
    f32, bf16, u32 = jnp.float32, jnp.bfloat16, jnp.uint32
    L, D = u_ref.shape
    N = are_ref.shape[1]
    S, Dm = x_ref.shape
    M = mem_ref.shape[0]
    H, Dh = wq_hbm.shape[1], wq_hbm.shape[2]
    T = _T
    nc = L // T
    nt_ = D // 128
    NG = H // grp
    LH = M + seg
    n_seg = S // seg
    nn = (((1,), (0,)), ((), ()))
    nt = (((1,), (1,)), ((), ()))

    u_copy = pltpu.make_async_copy(u_hbm, u_ref, sem.at[4])
    u_copy.start()
    for wi, wr in enumerate((wq_hbm, wk_hbm, wv_hbm)):
        w32 = wr.bitcast(u32)
        for hp in range(H // 2):
            pltpu.make_async_copy(w32.at[:, hp, :], stage.at[wi, hp], sem.at[wi]).start()
    wo_copy = pltpu.make_async_copy(wo_hbm.bitcast(u32), wos, sem.at[3])
    wo_copy.start()
    x_head = _X_HEAD * seg
    x_copy = pltpu.make_async_copy(x_hbm.at[:x_head], x_ref.at[:x_head], sem.at[5])
    x_copy.start()
    x_rest = pltpu.make_async_copy(x_hbm.at[x_head:], x_ref.at[x_head:], sem.at[6])

    a_list = cst["a_list"]
    dt_row = jnp.exp(ldt_ref[...].reshape(1, D).astype(f32)).astype(bf16).astype(f32)
    for j in range(nt_):
        cs = slice(j * 128, (j + 1) * 128)
        dt = jnp.broadcast_to(dt_row[:, cs], (N, 128)).T
        ld = lambda r: r[cs, :].astype(f32)
        par[0, cs] = dt * ld(are_ref)
        par[1, cs] = dt * ld(aim_ref)
        par[2, cs], par[3, cs] = _cmul(ld(cre_ref), ld(cim_ref), dt * ld(bre_ref), dt * ld(bim_ref))
    zs, xt, yt = (zs0, zs1), (xt0, xt1), (yt0, yt1)
    for r in xt:
        r[...] = jnp.zeros(r.shape, f32)
    n_grp = D // 8

    def bases(g, slot):
        r = pl.multiple_of(jnp.minimum(g, n_grp - 1) * 8, 8)
        ar, ai = par[0, pl.ds(r, 8), :], par[1, pl.ds(r, 8), :]
        e = jnp.exp(ar)
        zs[slot][0] = e * jnp.cos(ai)
        zs[slot][1] = e * jnp.sin(ai)

    def tables(g, slot):
        r = pl.multiple_of(jnp.minimum(g, n_grp - 1) * 8, 8)
        zq = {1: (zs[slot][0], zs[slot][1])}
        for q in range(2, 9):
            zq[q] = _cmul(*zq[q // 2], *zq[q - q // 2]) if q % 2 else _csqr(*zq[q // 2])
        yield zq[8][0]
        yb = {0: (jnp.ones((8, N), f32), jnp.zeros((8, N), f32)), 1: zq[8]}
        for b in range(_NB):
            if b > 1:
                yb[b] = _cmul(*yb[b // 2], *yb[b - b // 2]) if b % 2 else _csqr(*yb[b // 2])
            yt[slot][0, pl.ds(b, 8, stride=_SB), :] = yb[b][0]
            yt[slot][1, pl.ds(b, 8, stride=_SB), :] = yb[b][1]
            if b % 8 == 7:
                yield yb[b][1]
        zm = _csqr(*yb[_NB // 2])
        wm = (par[2, pl.ds(r, 8), :], par[3, pl.ds(r, 8), :])
        for idx, (m, q, _) in enumerate(a_list):
            if q == 0 and m > 0:
                wm = _cmul(*wm, *zm)
            v = wm if q == 0 else _cmul(*wm, *zq[q])
            xt[slot][0, pl.ds(idx, 8, stride=_SA), :] = v[0]
            xt[slot][1, pl.ds(idx, 8, stride=_SA), :] = -v[1]
            if idx % 7 == 6:
                yield v[1]

    def split(v):
        hi = pltpu.bitcast(pltpu.bitcast(v, u32) & u32(0xFFFF0000), f32)
        return hi, v - hi

    def after(v, tick):
        return v if tick is None else pltpu.bitcast(pltpu.bitcast(v, u32) | tick, f32)

    def tick_of(v):
        return pltpu.bitcast(v, u32) & zero[...]

    def mode_sum(g, slot, other=None):
        for i in range(8):
            tick = None if other is None else tick_of(next(other))
            lhs, rhs = [], []
            for part in range(2):
                xh, xl = split(xt[slot][part, i * _SA:i * _SA + _NA, :])
                y = [yt[slot][part, pl.ds(i * _SB + k, 8), :] for k in range(0, _NB, 8)]
                yh, yl = split(jnp.concatenate(y[:-1] + [after(y[-1], tick)], axis=0))
                lhs += [xh, xl, xh]
                rhs += [yh, yh, yl]
            kt[g, i * _SA:i * _SA + _NA, :] = jax.lax.dot_general(
                jnp.concatenate(lhs, axis=1), jnp.concatenate(rhs, axis=1), nt, preferred_element_type=f32)

    def regroup(j):
        hb = _NB // 2
        for idx, (_, _, dst) in enumerate(a_list):
            v = kt[pl.ds(j * 16, 16), pl.ds(idx, 8, stride=_SA), :].reshape(128, _NB).T
            if dst[1] is None:
                first = jax.lax.broadcasted_iota(jnp.int32, (hb, 128), 0) == 0
                kd[dst[0]:dst[0] + hb, :] = jnp.where(first, v[:hb], 0.0).astype(bf16)
            else:
                kd[dst[0]:dst[0] + hb, :] = v[:hb].astype(bf16)
                kd[dst[1]:dst[1] + hb, :] = v[hb:].astype(bf16)

    def forward(j):
        q, prev = T // 2, None
        cs = pl.ds(j * 128, 128)
        for c in range(nc):
            cur = jax.lax.dot_general(pltpu.bitcast(f_ref[0], bf16), u_ref[c * T:(c + 1) * T, cs],
                                      nn, preferred_element_type=f32)
            if prev is None:
                uh[j, c] = cur
            else:
                uh[j, c, 0:q] = cur[0:q] - prev[2 * q:3 * q]
                uh[j, c, q:2 * q] = cur[q:2 * q] + prev[3 * q:4 * q]
                uh[j, c, 2 * q:3 * q] = cur[2 * q:3 * q] + prev[0:q]
                uh[j, c, 3 * q:4 * q] = cur[3 * q:4 * q] - prev[q:2 * q]
            prev = cur
            if c % 3 == 0:
                yield
        for c, (mat, r0, w) in enumerate(cst["win"]):
            kh[j, c] = jax.lax.dot_general(pltpu.bitcast(f_ref[mat, :, :w], bf16), kd[r0:r0 + w, :],
                                           nn, preferred_element_type=f32)
            if c % 3 == 0:
                yield

    zero[...] = jnp.zeros(zero.shape, u32)
    bases(0, 0)
    bases(1, 1)
    list(tables(0, 0))

    def gen(i, carry):
        for k in range(2):
            g = 2 * i + k
            bases(g + 2, k)
            mode_sum(g, k, tables(g + 1, 1 - k))
        return carry
    jax.lax.fori_loop(0, n_grp // 2, gen, 0)
    u_copy.wait()

    for wi in range(3):
        pltpu.make_async_copy(stage.at[wi], stage.at[wi], sem.at[wi]).wait()

    def unpack_pair(item):
        wi, hp = item // (H // 2), item % (H // 2)
        ev = stage[wi, hp, pl.ds(0, Dm // 2, stride=2), :]
        od = stage[wi, hp, pl.ds(1, Dm // 2, stride=2), :]
        g, c0 = hp // (grp // 2), (hp % (grp // 2) * 6 + wi) * Dh
        wqkv[g, :, pl.ds(c0, Dh)] = (ev & u32(0xFFFF)) | (od << 16)
        wqkv[g, :, pl.ds(c0 + 3 * Dh, Dh)] = (ev >> 16) | (od & u32(0xFFFF0000))

    n_pair = 3 * H // 2
    per_tile = -(-n_pair // nt_)

    for j in range(nt_):
        regroup(j)
        for k, _ in enumerate(forward(j)):
            if k < per_tile and j * per_tile + k < n_pair:
                unpack_pair(j * per_tile + k)

    n_fb = T // 8

    def mac(j, fb):
        r = pl.multiple_of(fb * 8, 8)
        cb = 4
        for c0 in range(0, nc, cb):
            acc = [None] * cb
            for d in range(c0 + cb):
                tick = yield
                kr, ki = after(kh[j, d, pl.ds(r, 8), :], tick), after(kh[j, d, pl.ds(T + r, 8), :], tick)
                for c in range(max(c0, d), c0 + cb):
                    pr, pi = _cmul(kr, ki, uh[j, c - d, pl.ds(r, 8), :], uh[j, c - d, pl.ds(T + r, 8), :])
                    a_ = acc[c - c0]
                    acc[c - c0] = (pr, pi) if a_ is None else (a_[0] + pr, a_[1] + pi)
            for c in range(c0, c0 + cb):
                zb[j, c, pl.ds(r, 8), :] = acc[c - c0][0]
                zb[j, c, pl.ds(T + r, 8), :] = acc[c - c0][1]

    def inverse(c, j):
        yield
        cs = slice(j * 128, (j + 1) * 128)
        r = pl.multiple_of(c * T, T)
        z = zb[j, c].astype(bf16)
        y = jnp.concatenate([
            jax.lax.dot_general(pltpu.bitcast(g_ref[k * T // 4:(k + 1) * T // 4, :], bf16), z,
                                nn, preferred_element_type=f32) for k in range(2)], axis=0)
        skip = u_ref[pl.ds(r, T), cs].astype(f32) * dsk_ref[...].reshape(1, D)[:, cs].astype(f32)
        o_ref[pl.ds(r, T), cs] = (y + skip).astype(bf16)

    wo_copy.wait()
    x_copy.wait()
    x_rest.start()

    hbuf[0:M, :] = mem_ref[...].astype(f32)
    row = jax.lax.broadcasted_iota(jnp.int32, (LH, LH), 0)
    col = jax.lax.broadcasted_iota(jnp.int32, (LH, LH), 1)
    mask = (row < M) | (row >= col)
    scale = Dh ** -0.5

    def step(s, extra):
        r0 = pl.multiple_of(s * seg, seg)
        hbuf[M:LH, :] = x_ref[pl.ds(r0, seg), :].astype(f32)

        def qkv(g):
            outs = []
            for n0 in range(0, 3 * grp * Dh, 512):
                acc = None
                for k in range(Dm // 128):
                    w = pltpu.bitcast(wqkv[g, k * 64:(k + 1) * 64, n0:n0 + 512], bf16)
                    t = jax.lax.dot_general(hbuf[:, k * 128:(k + 1) * 128], w, nn, preferred_element_type=f32)
                    acc = t if acc is None else acc + t
                outs.append(acc)
            return jnp.concatenate(outs, axis=1)

        def probs(t):
            res = []
            for hh in range(grp):
                q, k, v = (t[:, (3 * hh + i) * Dh:(3 * hh + i + 1) * Dh] for i in range(3))
                sc = jax.lax.dot_general(q, k, nt, preferred_element_type=f32)
                sc = jnp.where(mask, sc, -1e9 / scale)
                e = jnp.exp2((sc - jnp.max(sc, axis=-1, keepdims=True)) * (scale * math.log2(math.e)))
                den = jnp.sum(e, axis=-1, keepdims=True)
                inv = pltpu.reciprocal(den, approx=True)
                res.append((e, v, inv * (2.0 - den * inv)))
            return res

        def mix(res):
            return jnp.concatenate(
                [jax.lax.dot_general(e, v, nn, preferred_element_type=f32) * inv for e, v, inv in res], axis=1)

        def oproj(og, g):
            nr = grp * Dh // 2
            w = pltpu.bitcast(wos[g * nr:(g + 1) * nr, :], bf16)
            return jax.lax.dot_general(og, w, nn, preferred_element_type=f32)

        acc, ts, ps, ogs = None, {}, {}, {}
        la, lp, lo = _LAGS
        for i in range(NG + lo):
            if i < NG:
                ts[i] = qkv(i)
            if 0 <= i - la < NG:
                ps[i - la] = probs(ts.pop(i - la))
            if 0 <= i - lp < NG:
                ogs[i - lp] = mix(ps.pop(i - lp))
            extra(i, ts.get(i))
            if 0 <= i - lo < NG:
                t = oproj(ogs.pop(i - lo), i - lo)
                acc = t if acc is None else acc + t
        extra(NG + lo, None)
        out = acc.astype(bf16)
        hbuf[0:M, :] = out[0:M].astype(f32)
        o_ref[pl.ds(r0, seg), D:] = out[M:LH]

    def interleave(gens, n_total, first, last):
        def chain():
            for g in gens:
                yield from g
        work = chain()
        next(work)

        def extra(i, t):
            if first <= i <= last:
                n, k = last - first + 1, i - first
                cnt = n_total * (k + 1) // n - n_total * k // n
                for m in range(cnt):
                    tick = None
                    if t is not None:
                        c0 = (m * (t.shape[1] // 128) // cnt) * 128
                        tick = tick_of(t[0:8, c0:c0 + 128])
                    try:
                        work.send(tick)
                    except StopIteration:
                        pass
        return extra

    s1 = n_seg - nc
    assert _X_HEAD < s1
    n_items = nt_ * n_fb
    per = -(-n_items // s1)

    def first(s, carry):
        pl.when(s == _X_HEAD)(x_rest.wait)
        items = [jnp.minimum(s * per + m, n_items - 1) for m in range(per)]
        step(s, interleave([mac(it // n_fb, it % n_fb) for it in items], per * 40, 0, NG - 1))
        return carry
    jax.lax.fori_loop(0, s1, first, 0)

    def out_copy(c):
        r = pl.multiple_of(c * T, T)
        return pltpu.make_async_copy(o_ref.at[pl.ds(r, T)], o_hbm.at[pl.ds(r, T)], osem.at[c])

    def finish(s, carry):
        c = s - s1
        step(s, interleave([inverse(c, j) for j in range(nt_)], nt_, NG + _LAGS[2] + 1 - nt_, NG + _LAGS[2]))
        out_copy(c).start()
        return carry
    jax.lax.fori_loop(s1, n_seg, finish, 0)
    for c in range(nc):
        out_copy(c).wait()


@functools.partial(jax.jit, static_argnames=("B_seg_len",))
def pallas_concat_heads__ssm_conv_s4__memory_aug_recurrent_mem_tr__prompt_kernel(
    A_u, A_A_re, A_A_im, A_B_re, A_B_im, A_C_re, A_C_im, A_log_dt, A_Dskip,
    B_x, B_mem0, B_Wq, B_Wk, B_Wv, B_Wo, B_seg_len,
):
    Bsz, L, D = A_u.shape
    N = A_A_re.shape[1]
    _, S, Dm = B_x.shape
    H, Dh = B_Wq.shape[1], B_Wq.shape[2]
    M = B_mem0.shape[1]
    assert Bsz == 1 and S == L and A_A_re.dtype == jnp.bfloat16
    grp = 4
    cst = _conv_constants(L)
    assert len(cst["a_list"]) <= _NA and N == 128
    f32, u32 = jnp.float32, jnp.uint32
    vm = pl.BlockSpec(memory_space=pltpu.VMEM)
    hbm = pl.BlockSpec(memory_space=pl.ANY)
    out = pl.pallas_call(
        functools.partial(_kernel, cst=cst, seg=B_seg_len, grp=grp),
        out_shape=jax.ShapeDtypeStruct((L, D + Dm), jnp.bfloat16),
        in_specs=[vm] * 11 + [hbm] * 6,
        out_specs=hbm,
        scratch_shapes=[
            pltpu.VMEM((H // grp, Dm // 2, 3 * grp * Dh), u32),
            pltpu.VMEM((H * Dh // 2, Dm), u32),
            pltpu.VMEM((M + B_seg_len, Dm), f32),
            pltpu.VMEM((3, H // 2, Dm, Dh), u32),
            pltpu.VMEM((L, D), jnp.bfloat16),
            pltpu.VMEM((S, Dm), jnp.bfloat16),
            pltpu.VMEM((L, D + Dm), jnp.bfloat16),
            pltpu.VMEM((4, D, N), f32),
            *[pltpu.VMEM((2, 8, N), f32)] * 2,
            *[pltpu.VMEM((2, 8 * _SA, N), f32)] * 2,
            *[pltpu.VMEM((2, 8 * _SB, N), f32)] * 2,
            pltpu.VMEM((D // 8, 8 * _SA, _NB), f32),
            pltpu.VMEM((cst["n_rows"], 128), jnp.bfloat16),
            pltpu.VMEM((D // 128, L // _T, 2 * _T, 128), f32),
            pltpu.VMEM((D // 128, L // _T, 2 * _T, 128), f32),
            pltpu.VMEM((D // 128, L // _T, 2 * _T, 128), f32),
            pltpu.VMEM((8, 128), u32),
            pltpu.SemaphoreType.DMA((7,)),
            pltpu.SemaphoreType.DMA((L // _T,)),
        ],
        compiler_params=pltpu.CompilerParams(vmem_limit_bytes=120 * 1024 * 1024),
        name="s4_rmt",
    )(A_A_re, A_A_im, A_B_re, A_B_im, A_C_re, A_C_im, A_log_dt, A_Dskip,
      B_mem0.reshape(M, Dm), cst["F"], cst["G"],
      A_u.reshape(L, D), B_x.reshape(S, Dm), B_Wq, B_Wk, B_Wv, B_Wo.reshape(H * Dh, Dm))
    return out.reshape(1, L, D + Dm)
```
